```python
import jax
import jax.numpy as jnp

def _softmax(x, axis=-1):
    return jax.nn.softmax(x, axis=axis)
def _gelu(x):
    return jax.nn.gelu(x, approximate=True)
def _silu(x):
    return jax.nn.silu(x)
def _sigmoid(x):
    return jax.nn.sigmoid(x)
def _layernorm(x, axis=-1, eps=1e-5):
    m = jnp.mean(x, axis=axis, keepdims=True)
    v = jnp.var(x, axis=axis, keepdims=True)
    return (x - m) / jnp.sqrt(v + eps)
def _scatter_add(tgt, idx, src, axis=0):
    return tgt.at[idx].add(src)
def _segment_sum(src, seg, n):
    return jax.ops.segment_sum(src, seg, n)
class _Rng:
    def __init__(self, key):
        self._k = key
    def _next(self):
        self._k, sub = jax.random.split(self._k)
        return sub
    def normal(self, shape):
        return jax.random.normal(self._next(), shape, dtype=jnp.bfloat16)
    def randint(self, lo, hi, shape):
        return jax.random.randint(self._next(), shape, lo, hi, dtype=jnp.int32)
    def uniform(self, shape, lo=0.0, hi=1.0):
        return jax.random.uniform(self._next(), shape, jnp.bfloat16, lo, hi)
    def permutation(self, n):
        return jax.random.permutation(self._next(), n)


kernel_name = 'standalone__gqa_block_cached__near_ridge'

def setup_inputs():
    _rng = _Rng(jax.random.key(int.from_bytes(__import__("os").urandom(4), "little")))
    _w = (lambda a: (lambda t: t.astype(jnp.bfloat16) if jnp.issubdtype(t.dtype, jnp.floating) else t)(jnp.asarray(a)))
    B, Sq, D = 16, 240, 640
    Hq, Hkv, Sk, Dh = 32, 32, 1024, 128
    assert Hq % Hkv == 0, (Hq, Hkv)
    return {
        "x": _w((lambda *s: _rng.normal(s) * 0.05)(B, Sq, D)),
        "k_cache": _w((lambda *s: _rng.normal(s) * 0.05)(B, Hkv, Sk, Dh)),
        "v_cache": _w((lambda *s: _rng.normal(s) * 0.05)(B, Hkv, Sk, Dh)),
        "wq": _w((lambda *s: _rng.normal(s) * 0.05)(D, Hq * Dh) * (D ** -0.5)),
        "wo": _w((lambda *s: _rng.normal(s) * 0.05)(Hq * Dh, D) * ((Hq * Dh) ** -0.5)),
    }

def reference(x, k_cache, v_cache, wq, wo):
    B, Sq, D = x.shape
    Hq, Dh = 32, 128
    Hkv = k_cache.shape[1]
    rep = Hq // Hkv
    q = (lambda x, *d: x.transpose(*d))((x @ wq).reshape(B, Sq, Hq, Dh), 0, 2, 1, 3)
    k = jnp.repeat(k_cache, rep, axis=1)
    v = jnp.repeat(v_cache, rep, axis=1)
    scores = jnp.einsum("bhqd,bhkd->bhqk", q, k) * (Dh ** -0.5)
    p = _softmax(scores, axis=-1)
    o = jnp.einsum("bhqk,bhkd->bhqd", p, v)
    return (lambda x, *d: x.transpose(*d))(o, 0, 2, 1, 3).reshape(B, Sq, Hq * Dh) @ wo
```

```python
import jax
import jax.numpy as jnp
from jax import lax
import jax.experimental.pallas as pl
import jax.experimental.pallas.tpu as pltpu

_G = 8
_HALF = 4
_LANES = 128
_LOG2E = 1.4426950408889634


@jax.jit
def pallas_standalone__gqa_block_cached__near_ridge_kernel(
    x: jax.Array,
    k_cache: jax.Array,
    v_cache: jax.Array,
    wq: jax.Array,
    wo: jax.Array,
):
    B, Sq, D = x.shape
    _, H, Sk, Dh = k_cache.shape
    G, HALF = _G, _HALF
    assert wq.shape == (D, H * Dh) and wo.shape == (H * Dh, D)
    assert Dh == _LANES and D % _LANES == 0 and Sq % 16 == 0 and H % G == 0
    nG, nD = H // G, D // _LANES
    NU = nG * B
    assert B & (B - 1) == 0 and B >= 2 + G + nD
    SP = -(-Sq // 32) * 32
    q_scale = Dh ** -0.5 * _LOG2E
    bf16 = jnp.bfloat16

    def kernel(x_hbm, k_hbm, v_hbm, wq_hbm, wo_hbm, o_hbm,
               kb, vb, wqb, wob, xb, qb, acc, ob,
               x_sem, k_sem, v_sem, wq_sem, wo_sem, o_sem, pro_sem):
        x32, k32, v32, wq32, wo32 = (
            r.bitcast(jnp.uint32) for r in (x_hbm, k_hbm, v_hbm, wq_hbm, wo_hbm))

        def pairs(row, n):
            return pl.ds(pl.multiple_of(row // 2, 16), n // 2)

        def load(buf, row, n):
            return pltpu.bitcast(buf[pairs(row, n), :], bf16)

        def lanes(c):
            return pl.ds(pl.multiple_of(c * _LANES, _LANES), _LANES)

        def split(u):
            return u >> (B.bit_length() - 1), u & (B - 1)

        def cache_copy(src, buf, u, h0, n, sem):
            g, b = split(u)
            return pltpu.make_async_copy(
                src.at[b, pairs((g * G + h0) * Sk, n * Sk)],
                buf.at[pairs(((u & 1) * G + h0) * Sk, n * Sk)], sem)

        def kv_copies(u):
            return [cache_copy(k32, kb, u, 0, G, k_sem.at[u & 1]),
                    cache_copy(v32, vb, u, 0, G, v_sem.at[u & 1])]

        def x_copies(b):
            return [pltpu.make_async_copy(
                x32.at[b, :, lanes(c)], xb.at[pairs((b * nD + c) * SP, Sq)], x_sem.at[b])
                for c in range(nD)]

        def wq_copy(g, h, sem):
            return pltpu.make_async_copy(
                wq32.at[:, lanes(g * G + h)], wqb.at[pairs(((g & 1) * G + h) * D, D)], sem)

        def wo_copy(g, c, sem):
            return pltpu.make_async_copy(
                wo32.at[pairs(g * G * Dh, G * Dh), lanes(c)],
                wob.at[pairs(((g & 1) * nD + c) * G * Dh, G * Dh)], sem)

        def out_copy(b):
            return pltpu.make_async_copy(ob.at[b], o_hbm.at[b], o_sem.at[0])

        def start(copies):
            for c in copies:
                c.start()

        def wait(copies):
            for c in copies:
                c.wait()

        def q_rows(u, h):
            return pl.ds(pl.multiple_of(((u & 1) * G + h) * SP, SP), Sq)

        def project_q(u, j):
            g, b = split(u)
            xv = jnp.concatenate(
                [load(xb, (b * nD + c) * SP, Sq) for c in range(nD)], axis=1)
            w = jnp.concatenate(
                [load(wqb, ((g & 1) * G + j * HALF + i) * D, D) for i in range(HALF)], axis=1)
            q = jnp.dot(xv, w, preferred_element_type=jnp.float32)
            q = (q * q_scale).astype(bf16)
            for i in range(HALF):
                qb[q_rows(u, j * HALF + i), :] = q[:, i * Dh:(i + 1) * Dh]

        class Unit:
            def __init__(self, u):
                self.u = u
                self.s, self.m, self.o, self.y = {}, {}, {}, None

            def scores(self, h):
                k = load(kb, ((self.u & 1) * G + h) * Sk, Sk)
                s = lax.dot_general(qb[q_rows(self.u, h), :], k, (((1,), (1,)), ((), ())),
                                    preferred_element_type=jnp.float32)
                self.s[h] = s
                self.m[h] = jnp.max(s, axis=-1, keepdims=True)

            def values(self, h):
                e = jnp.exp2(self.s[h] - self.m[h])
                l = jnp.sum(e, axis=-1, keepdims=True)
                if h < G - 2:
                    l = pltpu.roll(jnp.broadcast_to(l, (Sq, _LANES)), 1, 1)
                v = load(vb, ((self.u & 1) * G + h) * Sk, Sk)
                o = jnp.dot(e.astype(bf16), v, preferred_element_type=jnp.float32)
                r = pl.reciprocal(l, approx=True)
                r = r * (2.0 - l * r)
                self.o[h] = (o * r).astype(bf16)

            def heads(self, h0, h1):
                for h in range(h0, h1):
                    self.scores(h + 1)
                    self.values(h)

            def project_out(self, j):
                g, _ = split(self.u)
                o = jnp.concatenate([self.o[j * HALF + i] for i in range(HALF)], axis=1)
                w = jnp.concatenate(
                    [load(wob, (((g & 1) * nD + c) * G + j * HALF) * Dh, HALF * Dh)
                     for c in range(nD)], axis=1)
                y = jnp.dot(o, w, preferred_element_type=jnp.float32)
                self.y = y if self.y is None else self.y + y

        sems = iter(range(11))
        wq_lo, wq_hi = ([wq_copy(0, j * HALF + i, pro_sem.at[n]) for i in range(HALF)]
                        for j, n in ((0, next(sems)), (1, next(sems))))
        n = next(sems)
        wo_0 = [wo_copy(0, c, pro_sem.at[n]) for c in range(nD)]
        kc, vc = ({(u, j): cache_copy(src, buf, u, j * HALF, HALF, pro_sem.at[next(sems)])
                   for u in range(2) for j in range(2)}
                  for src, buf in ((k32, kb), (v32, vb)))
        start(x_copies(0) + wq_lo + wq_hi + [kc[0, 0], vc[0, 0]] + x_copies(1)
              + [kc[0, 1], vc[0, 1]] + wo_0 + [kc[1, 0], vc[1, 0]] + x_copies(2)
              + [kc[1, 1], vc[1, 1]] + x_copies(3))

        wait(x_copies(0) + wq_lo)
        project_q(0, 0)
        wait(wq_hi)
        project_q(0, 1)
        t = Unit(0)
        wait([kc[0, 0]])
        t.scores(0)
        t.scores(1)
        wait([vc[0, 0]] + x_copies(1))
        t.values(0)
        t.heads(1, HALF - 1)
        project_q(1, 0)
        wait([kc[0, 1], vc[0, 1]])
        t.heads(HALF - 1, G - 1)
        t.values(G - 1)
        project_q(1, 1)
        wait(wo_0)
        t.project_out(0)
        t.project_out(1)
        acc[0] = t.y

        t = Unit(1)
        wait([kc[1, 0], vc[1, 0]] + x_copies(2))
        t.scores(0)
        t.heads(0, HALF - 1)
        project_q(2, 0)
        wait([kc[1, 1], vc[1, 1]])
        start(kv_copies(2))
        t.heads(HALF - 1, G - 1)
        t.values(G - 1)
        t.project_out(0)
        project_q(2, 1)
        t.project_out(1)
        acc[1] = t.y

        def unit(u, carry):
            g, b = split(u)
            nxt = (g + 1) & 1

            @pl.when(u + 1 < B)
            def _():
                wait(x_copies(u + 1))

            @pl.when(b == B - 1)
            def _():
                for buf, rows, sem in ((wqb, G * D, wq_sem), (wob, nD * G * Dh, wo_sem)):
                    slab = buf.at[pairs(nxt * rows, rows)]
                    pltpu.make_async_copy(slab, slab, sem.at[nxt]).wait()

            wait(kv_copies(u))
            t = Unit(u)
            t.scores(0)
            t.scores(1)

            start(kv_copies(u + 1))

            @pl.when(u + 2 < B)
            def _():
                start(x_copies(u + 2))

            @pl.when((b >= 2) & (b < 2 + G) & (g + 1 < nG))
            def _():
                wq_copy(g + 1, b - 2, wq_sem.at[nxt]).start()

            @pl.when((b >= 2 + G) & (b < 2 + G + nD) & (g + 1 < nG))
            def _():
                wo_copy(g + 1, b - 2 - G, wo_sem.at[nxt]).start()

            @pl.when((g == nG - 1) & (b > 0))
            def _():
                out_copy(b - 1).start()

            t.values(0)
            t.heads(1, G - 1)
            t.values(G - 1)
            t.project_out(0)
            project_q(u + 1, 0)
            project_q(u + 1, 1)
            t.project_out(1)
            y = jnp.where(g == 0, 0.0, acc[b]) + t.y
            acc[b] = y
            ob[b] = y.astype(ob.dtype)
            return carry

        lax.fori_loop(2, NU - 1, unit, 0)

        wait(kv_copies(NU - 1))
        t = Unit(NU - 1)
        t.scores(0)
        t.scores(1)
        out_copy(B - 2).start()
        t.values(0)
        t.heads(1, G - 1)
        t.project_out(0)
        t.values(G - 1)
        t.project_out(1)
        ob[B - 1] = (acc[B - 1] + t.y).astype(ob.dtype)
        out_copy(B - 1).start()
        wait([out_copy(b) for b in range(B)])

    def staged(rows):
        return pltpu.VMEM((rows // 2, _LANES), jnp.uint32)

    hbm = pl.BlockSpec(memory_space=pl.ANY)
    dma = pltpu.SemaphoreType.DMA
    return pl.pallas_call(
        kernel,
        in_specs=[hbm] * 5,
        out_specs=hbm,
        out_shape=jax.ShapeDtypeStruct((B, Sq, D), x.dtype),
        scratch_shapes=[
            staged(2 * G * Sk),
            staged(2 * G * Sk),
            staged(2 * G * D),
            staged(2 * nD * G * Dh),
            staged(B * nD * SP),
            pltpu.VMEM((2 * G * SP, Dh), bf16),
            pltpu.VMEM((B, Sq, D), jnp.float32),
            pltpu.VMEM((B, Sq, D), x.dtype),
            dma((B,)), dma((2,)), dma((2,)), dma((2,)), dma((2,)), dma((1,)), dma((11,)),
        ],
        compiler_params=pltpu.CompilerParams(
            vmem_limit_bytes=100 * 1024 * 1024, disable_bounds_checks=True),
    )(x, k_cache.reshape(B, H * Sk, Dh), v_cache.reshape(B, H * Sk, Dh), wq, wo)
```
